```python
import os as _os
_os.environ.setdefault('JAX_PLATFORMS', 'cpu')
import jax
import jax.numpy as jnp

def _softmax(x, axis=-1):
    return jax.nn.softmax(x, axis=axis)

def _gelu(x):
    return jax.nn.gelu(x, approximate=True)

def _silu(x):
    return jax.nn.silu(x)

def _sigmoid(x):
    return jax.nn.sigmoid(x)

def _layernorm(x, axis=-1, eps=1e-05):
    m = jnp.mean(x, axis=axis, keepdims=True)
    v = jnp.var(x, axis=axis, keepdims=True)
    return (x - m) / jnp.sqrt(v + eps)

def _scatter_add(tgt, idx, src, axis=0):
    return tgt.at[idx].add(src)

def _segment_sum(src, seg, n):
    return jax.ops.segment_sum(src, seg, n)

class _Rng:

    def __init__(self, key):
        self._k = key

    def _next(self):
        self._k, sub = jax.random.split(self._k)
        return sub

    def normal(self, shape):
        return jax.random.normal(self._next(), shape, dtype=jnp.bfloat16)

    def randint(self, lo, hi, shape):
        return jax.random.randint(self._next(), shape, lo, hi, dtype=jnp.int32)

    def uniform(self, shape, lo=0.0, hi=1.0):
        return jax.random.uniform(self._next(), shape, jnp.bfloat16, lo, hi)

    def permutation(self, n):
        return jax.random.permutation(self._next(), n)
kernel_name = 'interleave_layers__ssm_conv_h3__mixer_gmlp__prompt'

def setup_inputs():
    _rng = _Rng(jax.random.key(int.from_bytes(__import__("os").urandom(4), "little")))
    _w = lambda a: (lambda t: t.astype(jnp.bfloat16) if jnp.issubdtype(t.dtype, jnp.floating) else t)(jnp.asarray(a))

    def _A_setup():
        B, S, D = (1, 2048, 1024)
        ks = 4
        return {'q': _w((lambda *s: _rng.normal(s) * 0.05)(B, S, D)), 'k': _w((lambda *s: _rng.normal(s) * 1.6)(B, S, D)), 'v': _w((lambda *s: _rng.normal(s) * 1.6)(B, S, D)), 'shift_k': _w((lambda *s: _rng.normal(s) * 1.6)(D, ks) * 0.5), 'ssm_k': _w((lambda *s: _rng.normal(s) * 1.6)(D, S) * (1.0 / S ** 0.5)), 'ssm_D': _w((lambda *s: _rng.normal(s) * 1.6)(D))}
    _A_in = _A_setup()

    def _B_setup():
        B, S, D, F = (1, 2048, 1024, 3584)
        Fh = F // 2
        return {'x': _w((lambda *s: _rng.normal(s) * 0.05)(B, S, D)), 'w_in': _w((lambda *s: _rng.normal(s) * 0.8)(D, 2 * Fh)), 'w_sp': _w(0.01 * (lambda *s: _rng.normal(s) * 0.8)(S, S)), 'b_sp': _w(1.0 + 0.01 * (lambda *s: _rng.normal(s) * 0.2)(S)), 'w_out': _w((lambda *s: _rng.normal(s) * 0.2)(Fh, D))}
    _B_in = _B_setup()
    return {'A_q': _A_in['q'], 'A_k': _A_in['k'], 'A_v': _A_in['v'], 'A_shift_k': _A_in['shift_k'], 'A_ssm_k': _A_in['ssm_k'], 'A_ssm_D': _A_in['ssm_D'], 'B_x': _B_in['x'], 'B_w_in': _B_in['w_in'], 'B_w_sp': _B_in['w_sp'], 'B_b_sp': _B_in['b_sp'], 'B_w_out': _B_in['w_out']}

def reference(A_q, A_k, A_v, A_shift_k, A_ssm_k, A_ssm_D, B_x, B_w_in, B_w_sp, B_b_sp, B_w_out):

    def _A_ref(q, k, v, shift_k, ssm_k, ssm_D):
        B, S, D = q.shape
        ks = shift_k.shape[-1]
        k_pad = jnp.pad(k, ((0, 0), (ks - 1, 0), (0, 0)))
        k_shift = jnp.zeros_like(k)
        for t in range(ks):
            k_shift = k_shift + k_pad[:, t:t + S, :] * shift_k[:, ks - 1 - t][None, None, :]
        kv = k_shift * v
        L = 2 * S
        kv_pad = jnp.pad(kv, ((0, 0), (0, S), (0, 0)))
        kf_pad = jnp.pad(ssm_k, ((0, 0), (0, S)))
        kv_f = (lambda x, axes=(-2, -1): jnp.fft.rfft2(x.astype(jnp.float32), axes=axes))(kv_pad[:, None, :, :], axes=(1, 2))
        kf_f = (lambda x, axes=(-2, -1): jnp.fft.rfft2(x.astype(jnp.float32), axes=axes))(kf_pad[:, None, :], axes=(1, 2))
        kf_f = (lambda x, *d: x.transpose(*d))(kf_f, 1, 2, 0)
        y_f = kv_f * kf_f[None, :, :, :]
        y = (lambda x, s, axes=(-2, -1): jnp.fft.irfft2(x, s=s, axes=axes).astype(jnp.bfloat16))(y_f, (1, L), axes=(1, 2))[:, 0, :S, :]
        y = y + kv * ssm_D[None, None, :]
        return q * y

    def _B_ref(x, w_in, w_sp, b_sp, w_out):
        B, S, D = x.shape
        F = w_in.shape[-1]
        Fh = F // 2
        z = _gelu(jnp.einsum('bsd,df->bsf', x, w_in))
        z1 = z[..., :Fh].copy()
        z2 = _layernorm(z[..., Fh:], axis=-1)
        g = jnp.einsum('ts,bsf->btf', w_sp, z2) + b_sp[None, :, None]
        return jnp.einsum('bsf,fd->bsd', z1 * g, w_out)
    x = A_q
    x = x + _A_ref(_layernorm(x, axis=-1), A_k, A_v, A_shift_k, A_ssm_k, A_ssm_D)
    x = x + _B_ref(_layernorm(x, axis=-1), B_w_in, B_w_sp, B_b_sp, B_w_out)
    x = x + _A_ref(_layernorm(x, axis=-1), A_k, A_v, A_shift_k, A_ssm_k, A_ssm_D)
    x = x + _B_ref(_layernorm(x, axis=-1), B_w_in, B_w_sp, B_b_sp, B_w_out)
    return x
```

```python
import functools
import math

import numpy as np
import jax
import jax.numpy as jnp
import jax.experimental.pallas as pl
import jax.experimental.pallas.tpu as pltpu

S = 2048
D = 1024
FH = 1792
F = 2 * FH
KS = 4
LANES = 128
NTILE = D // LANES
R = 16
N1 = S // R
TM = 256
NB = S // TM
TN = 256
EPS = 1e-5
F32 = jnp.float32
BF16 = jnp.bfloat16


class _V:
    def __init__(self, v, neg=False):
        self.v = v
        self.neg = neg

    def __neg__(self):
        return _V(self.v, not self.neg)


def _add(a, b):
    if a.neg == b.neg:
        return _V(a.v + b.v, a.neg)
    if b.neg:
        return _V(a.v - b.v)
    return _V(b.v - a.v)


def _sub(a, b):
    return _add(a, -b)


def _mul(a, b):
    return _V(a.v * b.v, a.neg != b.neg)


def _cadd(a, b):
    return (_add(a[0], b[0]), _add(a[1], b[1]))


def _csub(a, b):
    return (_sub(a[0], b[0]), _sub(a[1], b[1]))


def _cmul(a, b):
    return (_sub(_mul(a[0], b[0]), _mul(a[1], b[1])),
            _add(_mul(a[0], b[1]), _mul(a[1], b[0])))


_RS2 = float(np.sqrt(0.5))


def _rot(z, e):
    e = e % 16
    assert e % 2 == 0
    re, im = z
    if e % 4 == 2:
        a = _sub(re, im)
        b = _add(re, im)
        re, im = _V(a.v * _RS2, a.neg), _V(b.v * _RS2, b.neg)
        e -= 2
    for _ in range(e // 4):
        re, im = -im, re
    return (re, im)


def _split_fwd(a, e):
    if len(a) == 2:
        return [(a, e)]
    m = len(a) // 2
    hi = [_rot(z, e // 2) for z in a[m:]]
    p = [_cadd(x, y) for x, y in zip(a[:m], hi)]
    q = [_csub(x, y) for x, y in zip(a[:m], hi)]
    return _split_fwd(p, e // 2) + _split_fwd(q, e // 2 + 8)


def _merge_inv(res, e, n):
    if n == 2:
        return res.pop(0)
    m = n // 2
    p = _merge_inv(res, e // 2, m)
    q = _merge_inv(res, e // 2 + 8, m)
    lo = [_cadd(x, y) for x, y in zip(p, q)]
    hi = [_rot(_csub(x, y), -(e // 2)) for x, y in zip(p, q)]
    return lo + hi


def _cyc16(u, h):
    ru = _split_fwd(u, 0)
    rh = _split_fwd(h, 0)
    out = []
    for (a, e), (b, _) in zip(ru, rh):
        c0 = _cadd(_cmul(a[0], b[0]), _rot(_cmul(a[1], b[1]), e))
        c1 = _cadd(_cmul(a[0], b[1]), _cmul(a[1], b[0]))
        out.append([c0, c1])
    return _merge_inv(out, 0, R)


@functools.lru_cache(maxsize=None)
def _constants():
    n1 = np.arange(N1, dtype=np.float64)
    k1 = np.arange(N1, dtype=np.float64)
    g = np.zeros((R, 2 * N1, N1), np.float64)
    for n2 in range(R):
        ph = np.outer(2 * k1 + 1, R * n1 + n2) % (4 * S)
        th = 2.0 * np.pi * ph / (4 * S)
        g[n2, :N1] = np.cos(th)
        g[n2, N1:] = -np.sin(th)
    one = [(_V(1.0), _V(1.0)) for _ in range(R)]
    signs = _cyc16(one, one)
    ginv = np.transpose(g, (0, 2, 1)) / (8.0 * N1)
    for n2 in range(R):
        if signs[n2][0].neg:
            ginv[n2, :, :N1] *= -1.0
        if signs[n2][1].neg:
            ginv[n2, :, N1:] *= -1.0
    perm = np.zeros((LANES, LANES), np.float32)
    for n2 in range(R):
        for r in range(8):
            perm[n2 * 8 + r, R * r + n2] = 1.0
    return (g.astype(np.float32), ginv.astype(np.float32), perm)


def _gelu(x):
    c = math.sqrt(2.0 / math.pi)
    inner = x * (c + (c * 0.044715) * (x * x))
    hx = 0.5 * x
    return hx + hx * jnp.tanh(inner)


def _rowstats(x):
    n = x.shape[-1]
    m = jnp.sum(x, axis=-1, keepdims=True) * (1.0 / n)
    xc = x - m
    v = jnp.sum(xc * xc, axis=-1, keepdims=True) * (1.0 / n)
    return xc, jax.lax.rsqrt(v + EPS)


def _kernel(q_hbm, k_hbm, v_hbm, sk_ref, h_hbm, sd_ref, win_hbm, wsp_hbm,
            bsp_ref, wout_hbm, g_hbm, gi_hbm, perm_ref,
            o_hbm,
            kbuf, vbuf, hbuf, gbuf, gibuf, qbuf, win, wsp, wout,
            skT, bcol, ub, hb, au0, ah0, cb0, au1, ah1, cb1, ybuf, xbuf,
            z1, z2n, x2buf, z2raw, gz, xn_cur, xn_next, obuf, zero_ref,
            sem_k, sem_v, sem_h, sem_g, sem_q, sem_wi, sem_w, sem_o):
    def cp_k(j):
        return pltpu.make_async_copy(
            k_hbm.at[:, pl.ds(j * LANES, LANES)],
            kbuf.at[j, pl.ds(16, S), :], sem_k.at[j])

    def cp_v(j):
        return pltpu.make_async_copy(
            v_hbm.at[:, pl.ds(j * LANES, LANES)], vbuf.at[j], sem_v.at[j])

    def cp_h(j):
        return pltpu.make_async_copy(
            h_hbm.at[pl.ds(j * LANES, LANES), :], hbuf.at[j], sem_h.at[j])

    cp_g = pltpu.make_async_copy(g_hbm, gbuf, sem_g.at[0])
    cp_gi = pltpu.make_async_copy(gi_hbm, gibuf, sem_g.at[1])
    WCH = D // NTILE

    def cp_q(i):
        r = pl.ds(i * TM, TM)
        return pltpu.make_async_copy(q_hbm.at[r, :], qbuf.at[r, :], sem_q.at[i])

    def cp_win(j):
        r = pl.ds(j * WCH, WCH)
        return pltpu.make_async_copy(win_hbm.at[r, :], win.at[r, :], sem_wi.at[j])

    cp_wsp = pltpu.make_async_copy(wsp_hbm, wsp, sem_w.at[0])
    cp_wout = pltpu.make_async_copy(wout_hbm, wout, sem_w.at[1])

    cp_k(0).start()
    cp_v(0).start()
    cp_h(0).start()
    cp_g.start()
    cp_k(1).start()
    cp_v(1).start()
    cp_gi.start()
    cp_h(1).start()

    zero_ref[...] = jnp.zeros((8, LANES), jnp.uint32)
    for j in range(NTILE):
        kbuf[j, 0:16, :] = jnp.zeros((16, LANES), BF16)
    sel = (jax.lax.broadcasted_iota(jnp.int32, (8, KS), 0)
           == jax.lax.broadcasted_iota(jnp.int32, (8, KS), 1)).astype(BF16)
    skt = jax.lax.dot_general(sel, sk_ref[...], (((1,), (1,)), ((), ())),
                              preferred_element_type=F32)
    for j in range(NTILE):
        skT[j] = skt[:, j * LANES:(j + 1) * LANES]
    brow = jnp.broadcast_to(bsp_ref[...].astype(F32), (LANES, S))
    bcol[...] = brow.T

    kw = kbuf.bitcast(jnp.uint32)
    vw = vbuf.bitcast(jnp.uint32)
    himask = jnp.uint32(0xFFFF0000)

    def unpack(w):
        return (pltpu.bitcast(w << 16, F32), pltpu.bitcast(w & himask, F32))

    def orall(parts):
        while len(parts) > 1:
            parts = [parts[t] | parts[t + 1] if t + 1 < len(parts) else parts[t]
                     for t in range(0, len(parts), 2)]
        return parts[0]

    def tie0(xs, deps):
        if not deps:
            return xs
        d = orall(list(deps)) & zero_ref[...]
        corner = pltpu.bitcast(
            pltpu.bitcast(xs[0:16, 0:LANES], jnp.uint32) | d, BF16)
        if xs.shape[1] > LANES:
            corner = jnp.concatenate([corner, xs[0:16, LANES:]], axis=1)
        return jnp.concatenate([corner, xs[16:, :]], axis=0)

    CH = 16

    def s0_chunk(j, c):
        sk = skT[j]
        s0, s1, s2, s3 = (sk[t:t + 1, :] for t in range(KS))
        ks = {}
        toks = []
        for p in range(-2, 8):
            lo, hi = unpack(kw[j, pl.ds(8 + p + 8 * c * CH, CH, stride=8), :])
            ks[2 * p], ks[2 * p + 1] = lo, hi
            if p < 0:
                continue
            vs = unpack(vw[j, pl.ds(p + 8 * c * CH, CH, stride=8), :])
            for e in range(2):
                n2 = 2 * p + e
                ksh = (ks[n2] * s0 + ks[n2 - 1] * s1
                       + (ks[n2 - 2] * s2 + ks[n2 - 3] * s3))
                kv = (ksh * vs[e]).astype(BF16)
                ub[n2, c * CH:(c + 1) * CH, :] = kv
                if n2 % 4 == 3:
                    toks.append(pltpu.bitcast(kv, jnp.uint32))
        return orall(toks)

    def s0h_unit(j, jj, deps):
        perm = tie0(perm_ref[...], deps)
        a = jax.lax.dot_general(
            perm, hbuf[j, :, 256 * jj:256 * jj + 128],
            (((1,), (1,)), ((), ())), preferred_element_type=F32)
        b = jax.lax.dot_general(
            perm, hbuf[j, :, 256 * jj + 128:256 * jj + 256],
            (((1,), (1,)), ((), ())), preferred_element_type=F32)
        hb[:, 16 * jj:16 * jj + 16, :] = jnp.concatenate(
            [a.reshape(R, 8, LANES), b.reshape(R, 8, LANES)],
            axis=1).astype(BF16)

    def s1u_unit(n2, au, deps):
        au[n2] = jnp.dot(tie0(gbuf[n2], deps), ub[n2],
                         preferred_element_type=F32)

    def s1h_unit(j, n2, ah, deps):
        a = jnp.dot(tie0(gbuf[n2], deps), hb[n2], preferred_element_type=F32)
        if n2 == 0:
            a = jnp.concatenate([a[:N1] + sd_ref[j].astype(F32), a[N1:]], axis=0)
        ah[n2] = a

    def s2_group(i, au, ah, cb):
        r0 = i * 16
        r1 = N1 + i * 16
        outs = []
        for half in range(2):
            u = [(_V(au[n2, pl.ds(r0 + 8 * half, 8), :]),
                  _V(au[n2, pl.ds(r1 + 8 * half, 8), :])) for n2 in range(R)]
            h = [(_V(ah[n2, pl.ds(r0 + 8 * half, 8), :]),
                  _V(ah[n2, pl.ds(r1 + 8 * half, 8), :])) for n2 in range(R)]
            outs.append(_cyc16(u, h))
        toks = []
        for n2 in range(R):
            re = jnp.concatenate(
                [outs[0][n2][0].v, outs[1][n2][0].v], axis=0).astype(BF16)
            im = jnp.concatenate(
                [outs[0][n2][1].v, outs[1][n2][1].v], axis=0).astype(BF16)
            cb[n2, pl.ds(r0, 16), :] = re
            cb[n2, pl.ds(r1, 16), :] = im
            if n2 < 8:
                toks.append(pltpu.bitcast(re if n2 % 2 else im, jnp.uint32))
        return orall(toks)

    def s3_unit(j, n2, cb, deps):
        yv = jnp.dot(tie0(gibuf[n2], deps), cb[n2], preferred_element_type=F32)
        ybuf[j, pl.ds(n2, N1, stride=R), :] = yv

    def wait_kv(j):
        cp_k(j).wait()
        cp_v(j).wait()

    def stage(j, cur, nxt):
        au_c, ah_c, cb_c = cur
        au_n, ah_n, cb_n = nxt

        @pl.when(j + 1 < NTILE)
        def _():
            cp_h(j + 1).wait()

        @pl.when(j + 2 < NTILE)
        def _():
            wait_kv(j + 2)
            cp_h(j + 2).start()

        @pl.when(j + 3 < NTILE)
        def _():
            cp_k(j + 3).start()
            cp_v(j + 3).start()

        @pl.when(j + 2 >= NTILE)
        def _():
            cp_q(j + 2 - NTILE).start()

        cp_win(j).start()

        jm = jnp.maximum(j - 1, 0)
        j1 = jnp.minimum(j + 1, NTILE - 1)
        j2 = jnp.minimum(j + 2, NTILE - 1)
        mxu = ([(lambda d, n=n: s1u_unit(n, au_n, d), 1.0) for n in range(R)]
               + [(lambda d, n=n: s0h_unit(j1, n, d), 1.0) for n in range(8)]
               + [(lambda d, n=n: s3_unit(jm, n, cb_n, d), 1.0) for n in range(R)]
               + [(lambda d, n=n: s1h_unit(j1, n, ah_n, d), 1.0)
                  for n in range(R)])
        vpu = []
        order = ["2", "2", "2", "0", "0", "2", "0", "0", "2", "0", "0", "2",
                 "0", "0", "2", "2"]
        i2 = i0 = 0
        for o in order:
            if o == "2":
                vpu.append((lambda i=i2: s2_group(i, au_c, ah_c, cb_c), 1184.0))
                i2 += 1
            else:
                vpu.append((lambda c=i0: s0_chunk(j2, c), 340.0))
                i0 += 1
        tot_v = sum(w for _, w in vpu)
        pos = []
        acc = 0.0
        for _, w in vpu:
            acc += w
            pos.append(int(round(acc / tot_v * len(mxu))))
        k = 0
        for u, (fn, _) in enumerate(mxu):
            deps = []
            while k < len(vpu) and pos[k] <= u:
                deps.append(vpu[k][0]())
                k += 1
            fn(deps)
        while k < len(vpu):
            vpu[k][0]()
            k += 1

    bufs0 = (au0, ah0, cb0)
    bufs1 = (au1, ah1, cb1)
    cb1[...] = jnp.zeros(cb1.shape, BF16)
    wait_kv(0)
    cp_k(2).start()
    cp_v(2).start()
    for c in range(N1 // CH):
        s0_chunk(0, c)
    cp_h(0).wait()
    cp_g.wait()
    for n in range(8):
        s0h_unit(0, n, [])
    for n in range(R):
        s1u_unit(n, au0, [])
    wait_kv(1)
    toks = [s0_chunk(1, c) for c in range(N1 // CH)]
    for n in range(R):
        s1h_unit(0, n, ah0, [toks[n // 2]] if n % 2 == 1 else [])
    cp_gi.wait()

    def conv_pair(jj, carry):
        stage(2 * jj, bufs0, bufs1)
        stage(2 * jj + 1, bufs1, bufs0)
        return carry

    with jax.named_scope('conv'):
        jax.lax.fori_loop(0, NTILE // 2, conv_pair, 0)
    for n in range(R):
        s3_unit(NTILE - 1, n, cb1, [])

    for i in range(2, NB):
        cp_q(i).start()
    cp_wsp.start()
    cp_wout.start()

    RC = 16

    def rows(i):
        return pl.ds(pl.multiple_of(i * TM, TM), TM)

    def sub(i, c):
        return pl.ds(pl.multiple_of(i * TM + c * RC, RC), RC)

    def token(o):
        w = pltpu.bitcast(o, jnp.uint32)
        parts = [w[:, t * LANES:(t + 1) * LANES]
                 for t in range(w.shape[1] // LANES)]
        while len(parts) > 1:
            parts = [parts[t] | parts[t + 1] if t + 1 < len(parts) else parts[t]
                     for t in range(0, len(parts), 2)]
        return parts[0]

    def a_chunk(i, c, src_ref):
        r = sub(i, c)
        x = src_ref[r, :].astype(F32)
        y = jnp.concatenate([ybuf[j, r, :] for j in range(NTILE)], axis=1)
        xc, rs = _rowstats(x)
        x = x + (xc * rs) * y
        xbuf[r, :] = x
        xc, rs = _rowstats(x)
        o = (xc * rs).astype(BF16)
        xn_next[c * RC:(c + 1) * RC, :] = o
        return token(o)

    def z2_chunk(i, c, after):
        zr = z2raw[c * RC:(c + 1) * RC, :]
        d = after & zero_ref[...]
        d = jnp.concatenate([d] * (RC // 8), axis=0)
        corner = pltpu.bitcast(
            pltpu.bitcast(zr[:, 0:LANES], jnp.uint32) | d, F32)
        zr = jnp.concatenate([corner, zr[:, LANES:]], axis=1)
        zc, rs = _rowstats(zr)
        o = (zc * rs).astype(BF16)
        z2n[sub(i, c), :] = o
        return token(o)

    NCH = FH // TN
    NRC = TM // RC

    def spread(n_items, n_slots):
        return [list(range(s * n_items // n_slots, (s + 1) * n_items // n_slots))
                for s in range(n_slots)]

    def tie(xs, deps):
        if not deps:
            return xs
        nk = xs.shape[1] // LANES
        top = [xs[0:16, t * LANES:(t + 1) * LANES] for t in range(nk)]
        for m, d in enumerate(deps):
            kt = (m * nk) // len(deps)
            top[kt] = pltpu.bitcast(
                pltpu.bitcast(top[kt], jnp.uint32) | (d & zero_ref[...]), BF16)
        top = jnp.concatenate(top, axis=1)
        return jnp.concatenate([top, xs[16:, :]], axis=0)

    def mm_in(i, nxt, src_ref):
        xs = xn_cur[...]
        sa = spread(NRC, NCH)
        sz = spread(NRC, NCH - 2)
        nxt_deps = []
        deps = []
        for c in range(NCH):
            z = jnp.dot(tie(xs, deps), win[:, FH + c * TN:FH + (c + 1) * TN],
                        preferred_element_type=F32)
            z2raw[:, c * TN:(c + 1) * TN] = _gelu(z)
            deps = [a_chunk(nxt, t, src_ref) for t in sa[c]]
        for c in range(NCH):
            z = jnp.dot(tie(xs, deps), win[:, c * TN:(c + 1) * TN],
                        preferred_element_type=F32)
            z1[rows(i), c * TN:(c + 1) * TN] = _gelu(z).astype(BF16)
            deps = nxt_deps
            after = pltpu.bitcast(z[0:8, 0:LANES], jnp.uint32)
            nxt_deps = ([z2_chunk(i, t, after) for t in sz[c]]
                        if c < NCH - 2 else [])

    def mm_sp_out(i):
        ws = wsp[rows(i), :]
        bc = bcol[rows(i), :]
        bc = jnp.concatenate([bc] * (TN // LANES), axis=1)
        for c in range(FH // TN):
            g = jnp.dot(ws, z2n[:, c * TN:(c + 1) * TN],
                        preferred_element_type=F32) + bc
            gz[:, c * TN:(c + 1) * TN] = (
                z1[rows(i), c * TN:(c + 1) * TN].astype(F32) * g).astype(BF16)
        out = jnp.dot(gz[...], wout[...], preferred_element_type=F32)
        return xbuf[rows(i), :] + out

    def loop_in(src_ref, wait_q):
        for t in range(NRC):
            a_chunk(0, t, src_ref)

        def body(i, carry):
            nxt = jnp.minimum(i + 1, NB - 1)
            if wait_q:
                @pl.when(i + 1 < NB)
                def _():
                    cp_q(i + 1).wait()
            xn_cur[...] = xn_next[...]
            mm_in(i, nxt, src_ref)
            return carry

        with jax.named_scope("loop_in"):
            jax.lax.fori_loop(0, NB, body, 0)

    cp_q(0).wait()
    for j in range(NTILE):
        cp_win(j).wait()
    loop_in(qbuf, True)
    cp_wsp.wait()
    cp_wout.wait()

    def loop_b(i, carry):
        x2buf[rows(i), :] = mm_sp_out(i)
        return carry

    with jax.named_scope("loop_b"):
        jax.lax.fori_loop(0, NB, loop_b, 0)

    loop_in(x2buf, False)

    def cp_o(i):
        return pltpu.make_async_copy(obuf.at[rows(i), :], o_hbm.at[rows(i), :],
                                     sem_o.at[i])

    def loop_c(i, carry):
        obuf[rows(i), :] = mm_sp_out(i).astype(BF16)
        cp_o(i).start()
        return carry

    with jax.named_scope("loop_c"):
        jax.lax.fori_loop(0, NB, loop_c, 0)
    for i in range(NB):
        cp_o(i).wait()


@jax.jit
def pallas_interleave_layers__ssm_conv_h3__mixer_gmlp__prompt_kernel(
    A_q: jax.Array,
    A_k: jax.Array,
    A_v: jax.Array,
    A_shift_k: jax.Array,
    A_ssm_k: jax.Array,
    A_ssm_D: jax.Array,
    B_x: jax.Array,
    B_w_in: jax.Array,
    B_w_sp: jax.Array,
    B_b_sp: jax.Array,
    B_w_out: jax.Array,
):
    del B_x
    g, ginv, perm = _constants()
    hbm = pl.BlockSpec(memory_space=pl.ANY)
    vmem = pl.BlockSpec(memory_space=pltpu.VMEM)
    out = pl.pallas_call(
        _kernel,
        out_shape=jax.ShapeDtypeStruct((S, D), BF16),
        in_specs=[hbm, hbm, hbm, vmem, hbm, vmem, hbm, hbm, vmem, hbm,
                  hbm, hbm, vmem],
        out_specs=hbm,
        scratch_shapes=[
            pltpu.VMEM((NTILE, S + 16, LANES), BF16),
            pltpu.VMEM((NTILE, S, LANES), BF16),
            pltpu.VMEM((NTILE, LANES, S), BF16),
            pltpu.VMEM((R, 2 * N1, N1), BF16),
            pltpu.VMEM((R, N1, 2 * N1), BF16),
            pltpu.VMEM((S, D), BF16),
            pltpu.VMEM((D, F), BF16),
            pltpu.VMEM((S, S), BF16),
            pltpu.VMEM((FH, D), BF16),
            pltpu.VMEM((NTILE, 8, LANES), F32),
            pltpu.VMEM((S, LANES), F32),
            pltpu.VMEM((R, N1, LANES), BF16),
            pltpu.VMEM((R, N1, LANES), BF16),
            pltpu.VMEM((R, 2 * N1, LANES), F32),
            pltpu.VMEM((R, 2 * N1, LANES), F32),
            pltpu.VMEM((R, 2 * N1, LANES), BF16),
            pltpu.VMEM((R, 2 * N1, LANES), F32),
            pltpu.VMEM((R, 2 * N1, LANES), F32),
            pltpu.VMEM((R, 2 * N1, LANES), BF16),
            pltpu.VMEM((NTILE, S, LANES), F32),
            pltpu.VMEM((S, D), F32),
            pltpu.VMEM((S, FH), BF16),
            pltpu.VMEM((S, FH), BF16),
            pltpu.VMEM((S, D), F32),
            pltpu.VMEM((TM, FH), F32),
            pltpu.VMEM((TM, FH), BF16),
            pltpu.VMEM((TM, D), BF16),
            pltpu.VMEM((TM, D), BF16),
            pltpu.VMEM((S, D), BF16),
            pltpu.VMEM((8, LANES), jnp.uint32),
            pltpu.SemaphoreType.DMA((NTILE,)),
            pltpu.SemaphoreType.DMA((NTILE,)),
            pltpu.SemaphoreType.DMA((NTILE,)),
            pltpu.SemaphoreType.DMA((2,)),
            pltpu.SemaphoreType.DMA((NB,)),
            pltpu.SemaphoreType.DMA((NTILE,)),
            pltpu.SemaphoreType.DMA((2,)),
            pltpu.SemaphoreType.DMA((NB,)),
        ],
        compiler_params=pltpu.CompilerParams(
            vmem_limit_bytes=120 * 1024 * 1024),
    )(
        A_q.reshape(S, D), A_k.reshape(S, D), A_v.reshape(S, D),
        A_shift_k, A_ssm_k, A_ssm_D.reshape(NTILE, 1, LANES),
        B_w_in, B_w_sp, B_b_sp.reshape(1, S), B_w_out,
        jnp.asarray(g, BF16), jnp.asarray(ginv, BF16), jnp.asarray(perm, BF16),
    )
    return out.reshape(1, S, D)
```

```python
import functools
import math

import ml_dtypes
import numpy as np
import jax
import jax.numpy as jnp
import jax.experimental.pallas as pl
import jax.experimental.pallas.tpu as pltpu

S = 2048
D = 1024
FH = 1792
F = 2 * FH
KS = 4
LANES = 128
NTILE = D // LANES
P = 512
NP = S // P
NFFT = 2 * P
RF = 4
RI = 8
NG = 8
TM = 256
NB = S // TM
TN = 256
EPS = 1e-5
F32 = jnp.float32
BF16 = jnp.bfloat16
U32 = jnp.uint32


class _V:
    def __init__(self, v, neg=False):
        self.v = v
        self.neg = neg

    def __neg__(self):
        return _V(self.v, not self.neg)


def _add(a, b):
    if a.neg == b.neg:
        return _V(a.v + b.v, a.neg)
    if b.neg:
        return _V(a.v - b.v)
    return _V(b.v - a.v)


def _sub(a, b):
    return _add(a, -b)


def _mul(a, b):
    return _V(a.v * b.v, a.neg != b.neg)


def _cadd(a, b):
    return (_add(a[0], b[0]), _add(a[1], b[1]))


def _csub(a, b):
    return (_sub(a[0], b[0]), _sub(a[1], b[1]))


def _cmul(a, b):
    return (_sub(_mul(a[0], b[0]), _mul(a[1], b[1])),
            _add(_mul(a[0], b[1]), _mul(a[1], b[0])))


def _muli(z, sign):
    return (-z[1], z[0]) if sign > 0 else (z[1], -z[0])


def _pos(a):
    return _V(-a.v) if a.neg else a


def _dft4(a, sign):
    s0, d0 = _cadd(a[0], a[2]), _csub(a[0], a[2])
    s1, d1 = _cadd(a[1], a[3]), _muli(_csub(a[1], a[3]), sign)
    return [_cadd(s0, s1), _cadd(d0, d1), _csub(s0, s1), _csub(d0, d1)]


_RS2 = float(np.sqrt(0.5))


def _idft8(ye, yo):
    ev, od = _dft4(ye, 1), _dft4(yo, 1)
    tw = []
    for n, z in enumerate(od):
        if n % 2:
            a, b = _sub(z[0], z[1]), _add(z[0], z[1])
            z = (_V(a.v * _RS2, a.neg), _V(b.v * _RS2, b.neg))
        if n >= 2:
            z = _muli(z, 1)
        tw.append(z)
    return ([_cadd(x, y) for x, y in zip(ev, tw)]
            + [_csub(x, y) for x, y in zip(ev, tw)])


def _ones(n):
    return [(_V(1.0), _V(1.0)) for _ in range(n)]


_FWD_NEG = [(z[0].neg, z[1].neg) for z in _dft4(_ones(RF), -1)]
_INV_NEG = [(z[0].neg, z[1].neg) for z in _idft8(_ones(RF), _ones(RF))]


def _pack_rows(x):
    b = np.asarray(x, np.float32).astype(ml_dtypes.bfloat16).view(np.uint16)
    b = b.astype(np.uint32)
    return b[..., 0::2, :] | (b[..., 1::2, :] << 16)


@functools.lru_cache(maxsize=None)
def _constants():
    s8 = np.arange(8)
    kb = np.stack([2 * (8 * (g % 4) + s8) + g // 4 for g in range(NG)])
    col = np.arange(LANES)
    n1 = 16 * (col // 16) + 8 * (col % 2) + (col % 16) // 2
    g_f = np.zeros((RF, NG, 2, 2, 8, LANES), np.float64)
    for n2 in range(RF):
        for e in range(2):
            ph = ((2 * (kb + 128 * e) + 1)[:, :, None]
                  * (RF * n1 + n2)[None, None, :]) % (2 * NFFT)
            th = np.pi * ph / NFFT
            g_f[n2, :, e, 0] = np.cos(th)
            g_f[n2, :, e, 1] = -np.sin(th)
    g_f = g_f.reshape(RF, 2 * LANES, LANES)
    m1 = np.arange(P // RI)
    g_i = np.zeros((RI, P // RI, NG, 8, 2), np.float64)
    for n2 in range(RI):
        ph = ((RI * m1 + n2)[:, None, None] * (2 * kb + 1)[None]) % (2 * NFFT)
        th = np.pi * ph / NFFT
        g_i[n2, :, :, :, 0] = np.cos(th) * (-1.0 if _INV_NEG[n2][0] else 1.0)
        g_i[n2, :, :, :, 1] = -np.sin(th) * (-1.0 if _INV_NEG[n2][1] else 1.0)
    g_i = g_i.reshape(RI, P // RI, LANES) * (2.0 / NFFT)
    gw = _pack_rows(g_f).reshape(RF, NG, 2, 8, LANES)
    return np.concatenate(
        [x.reshape(-1, LANES) for x in
         (gw[0, :, 0], gw[2, :, 0], gw[1], gw[3], _pack_rows(g_i))], axis=0)


GI_ROWS = P // RI // 2
GI_OFF = 3 * LANES
DER_OFF = GI_OFF + RI * GI_ROWS
PERM_OFF = DER_OFF + LANES
CST_ROWS = PERM_OFF + LANES // 2


def _gelu2(x):
    c = math.sqrt(2.0 / math.pi)
    inner = x * (c + (c * 0.044715) * (x * x))
    return x + x * jnp.tanh(inner)


def _tilesum(x):
    parts = [x[:, t * LANES:(t + 1) * LANES] for t in range(x.shape[1] // LANES)]
    acc = parts[0]
    for p in parts[1:]:
        acc = acc + p
    return acc


def _rowstats(x, eps, tok):
    n = x.shape[-1]
    p = _tilesum(x)
    tok(p, 2.0)
    m = jnp.sum(p, axis=-1, keepdims=True) * (1.0 / n)
    xc = x - m
    p = _tilesum(xc * xc)
    tok(p, 3.0)
    v = jnp.sum(p, axis=-1, keepdims=True) * (1.0 / n)
    return xc, jax.lax.rsqrt(v + eps)


AHEAD = 50
WSTEP = [0,2,3,4,6,8,11]
WGRP = {1:[1],2:[2],3:[3],4:[4],5:[5,6],7:[7]}
HFIRST = 4
TF0 = 1280
MH = 128
TNI = 128
ZLAG = [256,256,256,128]
ZEND = 256
LSPAN = 768
S0SPAN = 2560
SSPAN = [768,704,896,832]
PSPAN = 100000
CPOS0 = 2
HPOS0 = 5
TF = 768
TL = [0,768,608,704]
HLEAD = 256
CLAG = 256
PAD = 4
AFIRST = 8
Q1AT = 2
QAT = 6
S0SPAN0 = 1024
AEXT = 2500
BOFF = 0.5
BSPAN = 0.9
FROW = 0
FD = 2
MEMQ = [[],[2,3],[2,3],[]]
OSPL = 1
CIAT = 2
S0TIE = [1,4,1.5,1]
LSPB = 1280
LB0 = 512
K0 = [0,2,3,4,6,8,8,11]


def _kernel(q_hbm, k_hbm, v_hbm, sk_hbm, h_hbm, sd_hbm, win_hbm, wsp_hbm,
            bsp_hbm, wout_hbm, cst_hbm,
            o_hbm,
            kw, vw, hbuf, cst, qbuf, win, wsp, wout,
            skT, bcol, ub, hb, cb, spec, ybuf, xbuf,
            z1, z2n, z2raw, gz, xn_cur, xn_next, obuf, zero_ref,
            sk_ref, sd_ref, bsp_ref, bsf, zs,
            sem_k, sem_v, sem_h, sem_c, sem_q, sem_wi, sem_w, sem_o):
    NCH = FH // TN
    PH, TH = P // 2, TM // 2
    q_w, k_w, v_w, h_w, win_w, wsp_w, wout_w, o_w = (
        r.bitcast(U32) for r in (q_hbm, k_hbm, v_hbm, h_hbm, win_hbm, wsp_hbm,
                                 wout_hbm, o_hbm))

    def cp_k(q, j):
        return pltpu.make_async_copy(
            k_w.at[pl.ds(q * PH, PH), pl.ds(j * LANES, LANES)],
            kw.at[j, pl.ds(8 + q * PH, PH), :], sem_k.at[q, j])

    def cp_v(q, j):
        return pltpu.make_async_copy(
            v_w.at[pl.ds(q * PH, PH), pl.ds(j * LANES, LANES)],
            vw.at[j, pl.ds(q * PH, PH), :], sem_v.at[q, j])

    def cp_h(q, j):
        return pltpu.make_async_copy(
            h_w.at[pl.ds(j * (LANES // 2), LANES // 2), pl.ds(q * P, P)],
            hbuf.at[j, :, pl.ds(q * P, P)], sem_h.at[q, j])

    cp_c = pltpu.make_async_copy(cst_hbm.at[0:GI_OFF, :], cst.at[0:GI_OFF, :],
                                 sem_c.at[0])
    cp_ci = pltpu.make_async_copy(cst_hbm.at[GI_OFF:DER_OFF, :],
                                  cst.at[GI_OFF:DER_OFF, :], sem_c.at[4])
    cp_sk = pltpu.make_async_copy(sk_hbm, sk_ref, sem_c.at[1])
    cp_sd = pltpu.make_async_copy(sd_hbm, sd_ref, sem_c.at[2])
    cp_bs = pltpu.make_async_copy(bsp_hbm, bsp_ref, sem_c.at[3])

    def cp_q(i):
        r = pl.ds(i * TH, TH)
        return pltpu.make_async_copy(q_w.at[r, :], qbuf.at[r, :], sem_q.at[i])

    def wcol(c):
        return (FH + c * TN) if c < NCH else (c - NCH) * TN

    def cp_win(c):
        cs = pl.ds(wcol(c), TN)
        return pltpu.make_async_copy(win_w.at[:, cs], win.at[:, cs],
                                     sem_wi.at[c])

    cp_wsp = pltpu.make_async_copy(wsp_w, wsp, sem_w.at[0])
    cp_wout = pltpu.make_async_copy(wout_w, wout, sem_w.at[1])

    queue = []

    def q_tile(q, j):
        queue.extend([(("k", q, j), cp_k(q, j), 1), (("v", q, j), cp_v(q, j), 1),
                      (("h", q, j), cp_h(q, j), 1)])

    queue.append((("sk",), cp_sk, 0))
    q_tile(0, 0)
    queue.append((("sd",), cp_sd, 0))
    queue.append((("bs",), cp_bs, 0))
    queue.append((("c",), cp_c, 2))
    for j in range(1, NTILE):
        q_tile(0, j)
        if j == CIAT:
            queue.append((("ci",), cp_ci, 1))
    queue.append((("q", 0), cp_q(0), 4))
    for c in range(2 * NCH):
        for t in range(NTILE):
            if K0[t] == c:
                q_tile(1, t)
        if c == Q1AT:
            queue.append((("q", 1), cp_q(1), 4))
        queue.append((("w", c), cp_win(c), 4))
    jobs = []
    for n in range(4):
        n0 = len(queue)
        queue.append((("q", n + 2), cp_q(n + 2), 4))
        for j in range(4 * (n % 2), 4 * (n % 2) + 4):
            q_tile(2 + n // 2, j)
        jobs.append([k for k, _, _ in queue[n0:]])
    qpos = {k: n for n, (k, _, _) in enumerate(queue)}
    state = {"started": 0}
    waited = set()

    def need(keys, ahead=AHEAD):
        last = max(qpos[k] for k in keys) if keys else state["started"] - 1
        n, acc = last + 1, 0
        while n < len(queue) and acc < ahead:
            acc += queue[n][2]
            n += 1
        for m in range(state["started"], n):
            queue[m][1].start()
        state["started"] = max(state["started"], n)
        for k in keys:
            queue[qpos[k]][1].wait()
            waited.add(k)

    need([])

    zero_ref[...] = jnp.zeros((8, LANES), U32)
    zs[0] = 0
    for j in range(NTILE):
        kw[j, 0:8, :] = jnp.zeros((8, LANES), U32)
    r2 = 2 * jax.lax.broadcasted_iota(jnp.int32, (LANES // 2, LANES), 0)
    dc = (jax.lax.broadcasted_iota(jnp.int32, (LANES // 2, LANES), 1)
          - RF * (r2 % (LANES // RF)) - r2 // (LANES // RF))
    cst[PERM_OFF:CST_ROWS, :] = jnp.where(
        dc == 0, jnp.uint32(0x3F80),
        jnp.where(dc == RF, jnp.uint32(0x3F800000), jnp.uint32(0)))
    need([("sk",)])
    skt = sk_ref[...].astype(F32)
    for j in range(NTILE):
        skT[j, 0:KS, :] = skt[:, j * LANES:(j + 1) * LANES]

    himask = jnp.uint32(0xFFFF0000)

    def bc(g, w):
        g = jnp.concatenate([g] * (w.shape[0] // 8), axis=0)
        return jnp.concatenate([g] * (w.shape[1] // LANES), axis=1)

    def lo16(w, gate=None):
        sh = jnp.uint32(16) if gate is None else bc(gate | jnp.uint32(16), w)
        return pltpu.bitcast(w << sh, F32)

    def hi16(w, gate=None):
        mk = himask if gate is None else bc(gate | himask, w)
        return pltpu.bitcast(w & mk, F32)

    def gated(x, gate):
        if gate is None:
            return x
        return pltpu.bitcast(pltpu.bitcast(x, U32) | bc(gate, x), F32)

    def as_bf16(w):
        return pltpu.bitcast(w, BF16)

    def as_u32(x):
        return pltpu.bitcast(x, U32)

    def pack2(a, b):
        return as_u32(pltpu.pack_elementwise([a, b], packed_dtype=BF16))

    def orall(parts):
        while len(parts) > 1:
            parts = [parts[t] | parts[t + 1] if t + 1 < len(parts) else parts[t]
                     for t in range(0, len(parts), 2)]
        return parts[0]

    def tied(w, deps):
        if not deps:
            return as_bf16(w)
        parts = []
        for r in range(w.shape[0] // 8):
            blk = w[8 * r:8 * r + 8, :]
            if r in deps:
                blk = blk | (deps[r] & zero_ref[...])
            parts.append(blk)
        return as_bf16(jnp.concatenate(parts, axis=0))

    def slot(q, j, t):
        return q * NTILE + j

    def s0_chunk(q, j, t, m, tok, gate):
        assert q > 1 or (("k", q, j) in waited and ("v", q, j) in waited)
        sk = skT[j, 0:KS, :]
        s0, s1, s2, s3 = (sk[x:x + 1, :] for x in range(KS))
        base = q * (P // 2) + 32 * m
        ks = {}
        for p in range(-2, 2):
            w = kw[j, pl.ds(8 + base + p, 16, stride=2), :]
            if p > -2:
                ks[2 * p] = lo16(w, gate)
            ks[2 * p + 1] = hi16(w, gate)
        toks = []
        for p in range(2):
            w = vw[j, pl.ds(base + p, 16, stride=2), :]
            for e, vv in enumerate((lo16(w, gate), hi16(w, gate))):
                n2 = 2 * p + e
                kv = (ks[n2] * s0 + ks[n2 - 1] * s1
                      + (ks[n2 - 2] * s2 + ks[n2 - 3] * s3)) * vv
                kv = pack2(kv[0:8], kv[8:16])
                ub[t % 2, n2, 8 * m:8 * m + 8, :] = kv
                toks.append(kv)
            tok(toks[-2] | toks[-1], 1.0)

    def s0h_unit(q, j, t, blk, deps):
        assert q > 1 or ("h", q, j) in waited
        c0 = q * P + blk * LANES
        a = jax.lax.dot_general(
            tied(cst[PERM_OFF:PERM_OFF + LANES // 2, :], deps),
            as_bf16(hbuf[j, :, c0:c0 + LANES]),
            (((1,), (1,)), ((), ())), preferred_element_type=F32)
        for n2 in range(RF):
            for hh in range(2):
                r = 32 * n2 + 16 * hh
                hb[t % 2, n2, 16 * blk + 8 * hh:16 * blk + 8 * hh + 8, :] = (
                    pack2(a[r:r + 8], a[r + 8:r + 16]))

    def s1_piece(t, g, out, mark, deps):
        for x in range(2):
            for n in range(RF):
                if n % 2:
                    r = LANES * (n + 1) // 2 + 16 * g
                    gm = cst[r:r + 16, :]
                else:
                    r = 32 * n + 8 * g
                    gm = jnp.concatenate(
                        [cst[r:r + 8, :], cst[DER_OFF + r:DER_OFF + r + 8, :]],
                        axis=0)
                out[x, n] = jnp.dot(
                    tied(gm, deps if x + n == 0 else {}),
                    as_bf16((ub, hb)[x][t % 2, n]), preferred_element_type=F32)
        return as_u32(out[0, 0][0:8]) if mark else None

    def s2_group(q, j, t, g, rawv, tok, gate):
        sg = 1 if g < NG // 2 else -1
        sl = slot(q, j, t)
        ys = []
        gz_ = as_u32(rawv[0, 0][0:8]) & zero_ref[...]
        mem = MEMQ[q]
        zo = zs[0] if mem else 0
        cur = {}
        for e in range(2):
            r = 32 * g + 16 * e
            for x in range(2):
                raw = [(_V(rawv[x, n][16 * e:16 * e + 8]),
                        _V(rawv[x, n][16 * e + 8:16 * e + 16]))
                       for n in range(RF)]
                if q == 0 and x == 1:
                    sd = sd_ref[...].astype(F32)[j:j + 1, :]
                    raw[0] = (_V(raw[0][0].v + sd), raw[0][1])
                cur[e, x] = _dft4(raw, -1)
                if q < NP - 1:
                    for n in range(RF):
                        spec[sl, x, n, r:r + 8, :] = cur[e, x][n][0].v
                        spec[sl, x, n, r + 8:r + 16, :] = cur[e, x][n][1].v
        for e in range(2):
            r = 32 * g + 16 * e

            def ld(s, x, n):
                return (_V(spec[s, x, n, r:r + 8, :]),
                        _V(spec[s, x, n, r + 8:r + 16, :]))

            ye = []
            for n in range(RF):
                own = [ld(sl + zo, x, n) if 2 * e + x in mem else cur[e, x][n]
                       for x in range(2)]
                us = [ld(slot(a, j, t), 0, n) for a in range(q)] + [own[0]]
                hs = [ld(slot(a, j, t), 1, n) for a in range(q)] + [own[1]]

                for b in range(q):
                    hs[b] = (_V(gated(hs[b][0].v, gz_)),
                             _V(gated(hs[b][1].v, gz_)))
                acc = _cmul(us[q], hs[0])
                for b in range(1, q + 1):
                    hp = _cadd(hs[b], _muli(hs[b - 1], sg))
                    acc = _cadd(acc, _cmul(us[q - b], hp))
                ye.append((_pos(acc[0]), _pos(acc[1])))
                if q:
                    gz_ = as_u32(acc[0].v) & zero_ref[...]
            ys.append(ye)
        c = _idft8(ys[0], ys[1])
        toks = []
        for n in range(RI):
            w = pack2(c[n][0].v, c[n][1].v)
            cb[t % 2, n, 8 * g:8 * g + 8, :] = w
            toks.append(w)
        tok(orall(toks[0::2]), 32.0)
        tok(orall(toks[1::2]), 40.0)

    def s3_unit(q, j, t, n2, deps):
        r0 = GI_OFF + n2 * GI_ROWS
        yv = jnp.dot(tied(cst[r0:r0 + GI_ROWS, :], deps),
                     as_bf16(cb[t % 2, n2]), preferred_element_type=F32)
        ybuf[j, pl.ds(q * P + n2, P // RI, stride=RI), :] = yv

    def h_units(q, j, t):
        return [(functools.partial(s0h_unit, q, j, t, b), 8) for b in range(4)]

    def p_step(t, g, out, mark=False):
        return (functools.partial(s1_piece, t, g, out, mark), [0, 16], 64)

    def c_units(q, j, t):
        return [(functools.partial(s3_unit, q, j, t, n), 4) for n in range(RI)]

    def run(steps, riders):
        t_end = np.cumsum([c for _, _, c in steps])
        slots = [(t_end[s] - c + ts, s, m) for s, (_, tl, c) in enumerate(steps)
                 for m, ts in enumerate(tl)]
        slots.sort()
        st = np.array([x[0] for x in slots])
        riders = sorted(riders, key=lambda r: r[1])
        due = [{} for _ in steps]
        k, gate, gates = 0, None, []
        for s in range(len(steps) + 1):
            while k < len(riders) and (s == len(steps)
                                       or riders[k][1] < t_end[s]):
                emit, t0, t1 = riders[k]
                toks = []
                gi = int(np.searchsorted(t_end, t0, side="right")) - 1
                emit(lambda v, c: toks.append((v, c)),
                     gates[gi] if gi >= 0 else None)
                tmin = t_end[s - 1] if s else 0.0
                tot = sum(c for _, c in toks)
                acc = 0.0
                for v, c in toks:
                    acc += c
                    at = int(np.searchsorted(
                        st, max(t0 + acc / tot * (t1 - t0), tmin)))
                    if at < len(slots):
                        if v.dtype != U32:
                            v = as_u32(v)
                        if v.shape[0] > 8:
                            v = v[0:8] | v[8:16]
                        _, s2, m = slots[at]
                        d = due[s2]
                        d[m] = (d[m] | v) if m in d else v
                k += 1
            if s < len(steps):
                mark = steps[s][0](due[s])
                if mark is not None:
                    gate = mark & zero_ref[...]
                gates.append(gate)

    def u_steps(units):
        out = []
        for g0 in range(0, len(units), 4):
            grp = units[g0:g0 + 4]
            nv = grp[0][1]

            def emit(deps, grp=grp):
                for n, (fn, _) in enumerate(grp):
                    fn(deps if n == 0 else {})
            out.append((emit, [16 * r for r in range(nv)], 16 * nv))
        return out

    def s0_items(q, j, t):
        return [functools.partial(s0_chunk, q, j, t, m) for m in range(8)]

    def kv_keys(q, j):
        return [("k", q, j), ("v", q, j)]

    def w_step(keys):
        def emit(deps):
            with jax.named_scope("w_" + "".join(str(x) for x in keys[0])):
                need(keys)
        return (emit, [], 0)

    def rebuild(deps):
        odd = (jax.lax.broadcasted_iota(jnp.int32, (8, LANES), 1) >> 1) & 1
        im = jax.lax.broadcasted_iota(jnp.int32, (8, LANES), 0) >> 2
        for n, flip in ((0, odd), (2, odd ^ im)):
            mk = jnp.where(flip == 1, jnp.uint32(0x80008000), jnp.uint32(0))
            for g in range(NG):
                r = 32 * n + 8 * g
                w = cst[r:r + 8, :]
                w = pltpu.roll(w, 4, 0) if n else w
                cst[DER_OFF + r:DER_OFF + r + 8, :] = w ^ mk

    def prefix0():
        steps, riders, now = [], [], 0.0
        for t in range(-1, NTILE + 1):
            keys = []
            for tt in WGRP.get(t + 1, []):
                keys += kv_keys(0, tt) + [("h", 0, tt)]
            if t == -1:
                steps.append(w_step(kv_keys(0, 0)))
                keys = [("h", 0, 0), ("sd",), ("bs",), ("c",)]
                for fn in s0_items(0, 0, 0):
                    riders.append((fn, now, now))
                steps.append((lambda deps: None, [], 1))
                now += 1
                steps.append(w_step(keys))
                steps.append((rebuild, [], 0))
                steps += u_steps(h_units(0, 0, 0))
                now += 128
                continue
            if t == 1:
                keys += [("ci",)]
            if t == QAT:
                keys += [("q", 0)]
            if keys:
                steps.append(w_step(keys))
            s0 = s0_items(0, t + 1, t + 1) if t + 1 < NTILE else []
            for g in range(NG):
                if t < NTILE:
                    out = {}
                    steps.append(p_step(t, g, out, True))
                    now += 64
                    riders.append((functools.partial(
                        s2_group, 0, t, t, g, out), now, now + PSPAN))
                if g == CPOS0 and t >= 1:
                    steps += u_steps(c_units(0, t - 1, t - 1))
                    now += 128
                if g == HPOS0 and s0:
                    steps += u_steps(h_units(0, t + 1, t + 1))
                    now += 128
                if s0 and g < 4:
                    for fn in s0[2 * g:2 * g + 2]:
                        riders.append((fn, now, now + PSPAN))
        return steps, riders

    RC = 16
    NRC = TM // RC
    NH = TM // MH

    def rows(i):
        return pl.ds(pl.multiple_of(i * TM, TM), TM)

    def wrows(i):
        return pl.ds(pl.multiple_of(i * TH, TH), TH)

    def cat(parts):
        return jnp.concatenate(parts, axis=1)

    def load_q(i, c, gate):
        assert not isinstance(i, int) or ("q", i) in waited
        w = qbuf[pl.ds(pl.multiple_of(i * TH + c * 8, 8), 8), :]
        return jnp.concatenate([lo16(w, gate), hi16(w, gate)], axis=0)

    def corner(x, gate):
        return cat([gated(x[:, 0:LANES], gate), x[:, LANES:]])

    def load_out(i, c, tiles):
        r0 = 32 * (c // 2) + c % 2
        return jnp.concatenate(
            [cat([spec[i, j // RF, j % RF, pl.ds(r0 + 2 * e, 8, stride=4), :]
                  for j in tiles]) for e in range(2)], axis=0)

    def load_x2(i, c, gate):
        r = pl.ds(pl.multiple_of(i * TM + c * RC, RC), RC)
        return corner(xbuf[r, :], gate) + load_out(i, c, range(NTILE))

    def a_chunk(i, c, load, xrow, xn_ref, nrow, tok, gate):
        x = load(i, c, gate)
        r0 = i * TM + c * RC
        y = jnp.concatenate(
            [cat([ybuf[j, pl.ds(r0 + e, 8, stride=2), :] for j in range(NTILE)])
             for e in range(2)], axis=0)
        xc, rs = _rowstats(x, EPS, tok)
        x = x + (xc * rs) * y
        xbuf[pl.ds(pl.multiple_of(xrow, RC), RC), :] = x
        xc, rs = _rowstats(x, EPS, tok)
        o = xc * rs
        o = pack2(o[0:8], o[8:16])
        xn_ref[pl.ds(pl.multiple_of(nrow, 8), 8), :] = o
        tok(orall([o[:, t * LANES:(t + 1) * LANES] for t in range(NTILE)]), 2.0)

    def z2_chunk(i, c, tok, gate):
        zr = jnp.concatenate(
            [cat([z2raw[t, pl.ds(c * RC + e, 8, stride=2), :]
                  for t in range(FH // LANES)]) for e in range(2)], axis=0)
        zc, rs = _rowstats(corner(zr, gate), 4.0 * EPS, tok)
        o = zc * (0.5 * rs)
        o = pack2(o[0:8], o[8:16])
        z2n[pl.ds(pl.multiple_of(i * TH + c * 8, 8), 8), :] = o
        tok(orall([o[:, t * LANES:(t + 1) * LANES]
                   for t in range(FH // LANES)]), 2.0)

    def tie(w, deps):
        if not deps:
            return as_bf16(w)
        nr = w.shape[0] // 8
        out = []
        for r in range(nr):
            blk = w[8 * r:8 * r + 8, :]
            hit = {4 * (m // nr): d for m, d in deps.items() if m % nr == r}
            if hit:
                blk = cat([
                    blk[:, t * LANES:(t + 1) * LANES] | (hit[t] & zero_ref[...])
                    if t in hit else blk[:, t * LANES:(t + 1) * LANES]
                    for t in range(w.shape[1] // LANES)])
            out.append(blk)
        return as_bf16(jnp.concatenate(out, axis=0))

    def pack32(g):
        return jnp.concatenate(
            [pack2(g[r + h:r + h + 8], g[r + h + 16:r + h + 24])
             for r in range(0, g.shape[0], 32) for h in (0, 8)], axis=0)

    def unpack32(w):
        parts = []
        for r in range(0, w.shape[0], 16):
            a, b = w[r:r + 8], w[r + 8:r + 16]
            parts += [lo16(a), lo16(b), hi16(a), hi16(b)]
        return jnp.concatenate(parts, axis=0)

    def mm_in(i, xs_ref, xs_row, a_riders, conv=None, pre=None, prefix=None,
              more=()):
        HW = MH // 2
        NT = F // TNI

        def m_step(c, h, deps):
            col = wcol(c * TNI // TN) + (c * TNI) % TN
            assert pre is None or ("w", c * TNI // TN) in waited
            xs = xs_ref[pl.ds(xs_row + h * HW, HW), :]
            z = jnp.dot(tie(xs, deps), as_bf16(win[:, col:col + TNI]),
                        preferred_element_type=F32)
            gl = _gelu2(z)
            if col >= FH:
                for t in range(TNI // LANES):
                    z2raw[(col - FH) // LANES + t, h * MH:(h + 1) * MH, :] = (
                        gl[:, t * LANES:(t + 1) * LANES])
            else:
                r0 = pl.multiple_of(i * TH + h * HW, HW)
                gl = pack32(gl)
                z1[pl.ds(r0, HW), col:col + TNI] = gl
            return as_u32(z[0:8, 0:LANES])

        q, tiles, t_first, t_last = conv if conv is not None else (0, [], 0, 0)
        mc = 2 * MH * TNI // LANES
        tm_all = NT * NH * mc
        extra = []
        npc = max(len(tiles) * NG, 1)
        dt = (tm_all - t_last - t_first) / (npc - 1 if npc > 1 else 1)
        outs = {}
        for t, j in enumerate(tiles):
            tp = t_first + t * NG * dt
            extra.append((tp - HLEAD, ("h", t), u_steps(h_units(q, j, t))))
            for g in range(NG):
                outs[t, g] = {}
                extra.append((tp + g * dt, ("p", t, g),
                              [p_step(t, g, outs[t, g])]))
            extra.append((min(tp + NG * dt + CLAG, tm_all), ("c", t),
                          u_steps(c_units(q, j, t))))
        extra.sort(key=lambda e: e[0])
        steps, at, mi, k = [], {}, 0, 0
        mt = [16 * m for m in range(2 * MH // 16)]
        order = [(c, h) for c in range(NT) for h in range(NH)]
        riders, tb = [], 0.0
        if prefix is not None:
            steps, riders = prefix
            tb = float(sum(c for _, _, c in steps))
            order = ([(c, h) for h in range(NH) for c in range(HFIRST)]
                     + order[NH * HFIRST:])
            for m, fn in enumerate(q_riders(0, xn_cur)):
                if m < AFIRST:
                    riders.append((fn, tb, 1e9))
                else:
                    t0 = tb + 1 + (m - AFIRST) * (HFIRST * mc - LSPAN) / 8
                    riders.append((fn, t0, t0 + LSPAN))
            steps.append((lambda deps: None, [], 1))
            tb += 1
        for n, (c, h) in enumerate(order):
            if True:
                if pre is not None and n % (NH * TN // TNI) == 0:
                    keys = pre(n // (NH * TN // TNI))
                    if keys:
                        steps.append(w_step(keys))
                        for t in range(NTILE):
                            if ("k", 1, t) in keys:
                                at["k", t] = len(steps) - 1
                        if ("q", 1) in keys:
                            at["q1"] = len(steps) - 1
                steps.append((functools.partial(m_step, c, h), mt, mc))
                mi += mc
                if 2 * mi == tm_all:
                    at["z"] = len(steps) - 1
                while k < len(extra) and extra[k][0] < mi + mc / 2:
                    steps += extra[k][2]
                    at[extra[k][1]] = len(steps) - 1
                    k += 1
        t_end = np.cumsum([c for _, _, c in steps])
        tz, te = t_end[at["z"]] + ZLAG[q], t_end[-1] - ZEND
        na = len(a_riders)
        ta = t_end[at["q1"]] if prefix is not None else 0.0
        for m, fn in enumerate(a_riders):
            t0 = ta + m / na * (tz + (AEXT if prefix else 0) - LSPAN - ta)
            riders.append((fn, t0, t0 + LSPAN))
        for m, fn in enumerate(more):
            t0 = (m + BOFF) / len(more) * BSPAN * te
            riders.append((fn, t0, t0))
        for c in range(NRC):
            t0 = tz + c / (NRC - 1) * (te - tz - LSPAN)
            riders.append((functools.partial(z2_chunk, i, c), t0, t0 + LSPAN))
        for t, j in enumerate(tiles):
            t1 = t_end[at["p", t, 0] - 1]
            t0 = max(t1 - (S0SPAN if prefix is None else S0SPAN0),
                     t_end[at["p", t - 2, NG - 1]] if t >= 2 else 0.0,
                     t_end[at["k", t]] if prefix is not None else 0.0)
            for m, fn in enumerate(s0_items(q, j, t)):
                riders.append((fn, t0 + m / 8 * (t1 - t0),
                               t0 + (m + S0TIE[q]) / 8 * (t1 - t0)))
            for g in range(NG):
                t0 = t_end[at["p", t, g]]
                riders.append((functools.partial(
                    s2_group, q, j, t, g, outs[t, g]), t0, t0 + SSPAN[q]))
        run(steps, riders)

    def mm_sp_out(i, riders, fin):
        def sp_step(c, deps):
            ws = wsp[wrows(i), :]
            bc = bcol[rows(i), :]
            g = jnp.dot(tie(ws, deps), as_bf16(z2n[:, c * TN:(c + 1) * TN]),
                        preferred_element_type=F32)
            gb = g + cat([bc] * (TN // LANES))
            gz[:, c * TN:(c + 1) * TN] = pack32(
                unpack32(z1[wrows(i), c * TN:(c + 1) * TN]) * gb)
            return as_u32(g[0:8, 0:LANES])

        def out_step(c, deps):
            out = jnp.dot(as_bf16(gz[...]),
                          as_bf16(wout[:, c * TN:(c + 1) * TN]),
                          preferred_element_type=F32)
            tl = range(c * (TN // LANES), (c + 1) * (TN // LANES))
            for j in tl:
                spec[i, j // RF, j % RF, 0:TM, :] = out[
                    :, (j - tl[0]) * LANES:(j - tl[0] + 1) * LANES]
            if fin:
                def gate(gr):
                    return as_u32(out[32 * gr + FROW:32 * gr + FROW + 8,
                                      TN - LANES:]) & zero_ref[...]
                ng = TM // 32
                for r in range(NRC):
                    gr = r // 2 + FD
                    if gr >= ng and c:
                        fin_chunk(c - 1, r, gate(gr - ng))
                for r in range(NRC):
                    gr = r // 2 + FD
                    if gr < ng or c == D // TN - 1:
                        fin_chunk(c, r, gate(gr) if gr < ng else None)

        def fin_chunk(c, r, gate):
            tl = range(c * (TN // LANES), (c + 1) * (TN // LANES))
            x = gated(
                xbuf[pl.ds(pl.multiple_of(i * TM + r * RC, RC), RC),
                     c * TN:(c + 1) * TN], gate) + load_out(i, r, tl)
            obuf[pl.ds(pl.multiple_of(i * TH + r * 8, 8), 8),
                 c * TN:(c + 1) * TN] = pack2(x[0:8], x[8:16])

        mt = [32 * m for m in range(64)]
        steps = ([(functools.partial(sp_step, c), mt, 2048) for c in range(NCH)]
                 + [(functools.partial(out_step, c), [], 1792)
                    for c in range(D // TN)])
        span = NCH * 2048 - LSPB - LB0
        run(steps, [(fn, LB0 + m / NRC * span, LB0 + m / NRC * span + LSPB)
                    for m, fn in enumerate(riders)])

    def q_riders(nxt, dst=xn_next):
        return [functools.partial(
            a_chunk, nxt, c, load_q, nxt * TM + c * RC, dst, c * 8)
            for c in range(NRC)]

    def pre0(c):
        keys = [("q", 1)] if c == Q1AT else []
        if c in WSTEP:
            nxt = ([x for x in WSTEP if x > c] + [2 * NCH])[0]
            for cc in range(c, nxt):
                keys.append(("w", cc))
                for t in range(NTILE):
                    if K0[t] == cc:
                        keys += kv_keys(1, t) + [("h", 1, t)]
        return keys

    with jax.named_scope("sec_0"):
        mm_in(0, xn_cur, 0, q_riders(1), (1, list(range(NTILE)), TF0, TL[1]),
              pre0, prefix0())
    need(jobs[0], ahead=10 ** 6)

    bsf[...] = 0.5 * bsp_ref[...].astype(F32)

    def bcol_piece(t, tok=None, gate=None):
        row = gated(jnp.broadcast_to(bsf[pl.ds(t, 1), :], (8, LANES)), gate)
        bcol[pl.ds(pl.multiple_of(t * LANES, LANES), LANES), :] = (
            jnp.concatenate([row] * (LANES // 8), axis=0).T)

    def make_bcol():
        for t in range(S // LANES):
            bcol_piece(t)

    for _ in range(PAD):
        pl.when(zs[0] != 0)(make_bcol)

    def conv_body(q):
        def body(i, carry):
            base = 4 * (i - (2 * q - 3))
            xn_cur[...] = xn_next[0:TH, :]
            mm_in(i, xn_cur, 0, q_riders(i + 1),
                  (q, [base + t for t in range(4)], TF, TL[q]))
            if q == 2:
                pl.when(base == 0)(lambda: need(jobs[1]))
            return carry
        return body

    with jax.named_scope("sec_2"):
        jax.lax.fori_loop(1, 3, conv_body(2), 0)
    for cp in (cp_q(6), cp_q(7), cp_wout):
        cp.start()
    need(jobs[2] + jobs[3])
    with jax.named_scope("sec_3"):
        jax.lax.fori_loop(3, 5, conv_body(3), 0)
    cp_wsp.start()
    cp_q(6).wait()
    cp_q(7).wait()

    def plain_body(i, carry):
        xn_cur[...] = xn_next[0:TH, :]
        mm_in(i, xn_cur, 0, q_riders(jnp.minimum(i + 1, NB - 1)),
              more=[functools.partial(
                  bcol_piece, jnp.minimum(6 * (i - 5) + m, S // LANES - 1))
                  for m in range(6)])
        return carry

    with jax.named_scope("sec_5"):
        jax.lax.fori_loop(5, NB, plain_body, 0)

    cp_wsp.wait()
    cp_wout.wait()
    assert len(waited) == len(queue) == state["started"]

    def loop_b(i, carry):
        src = jnp.maximum(i - 1, 0)
        dst = jnp.where(i > 0, i - 1, NB)
        mm_sp_out(i, [functools.partial(
            a_chunk, src, c, load_x2, dst * TM + c * RC, qbuf,
            dst * TH + c * 8) for c in range(NRC)], False)
        return carry

    with jax.named_scope("sec_b"):
        jax.lax.fori_loop(0, NB, loop_b, 0)

    NL = 4

    def load_x2_last(i, c, gate):
        ii, k = c
        r = pl.ds(pl.multiple_of(i * TM + (NL * ii + k) * RC, RC), RC)
        r0 = 32 * (NL // 2) * ii + 32 * (k // 2) + k % 2
        out = jnp.concatenate(
            [cat([spec[i, j // RF, j % RF, pl.ds(r0 + 2 * e, 8, stride=4), :]
                  for j in range(NTILE)]) for e in range(2)], axis=0)
        return corner(xbuf[r, :], gate) + out

    def loop_in2(i, carry):
        @pl.when(i == NB - 1)
        def _():
            qbuf[(NB - 1) * TH:NB * TH, :] = xn_next[0:TH, :]
        live = i < NRC // NL
        ii = jnp.minimum(i, NRC // NL - 1)
        riders = []
        for k in range(NL):
            c = NL * ii + k
            riders.append(functools.partial(
                a_chunk, NB - 1, c,
                lambda b, _, gt, k=k: load_x2_last(b, (ii, k), gt),
                jnp.where(live, (NB - 1) * TM + c * RC, S + RC), xn_next,
                jnp.where(live, c * 8, TH)))
        mm_in(i, qbuf, pl.multiple_of(i * TH, TH), riders)
        return carry

    with jax.named_scope("sec_i"):
        jax.lax.fori_loop(0, NB, loop_in2, 0)

    ocut = [(NB - 1) * TH] + [(NB - 1) * TH + (n + 1) * TH // OSPL
                              for n in range(OSPL)]

    def cp_o(n):
        r0 = ocut[n - 1] if n else 0
        r = pl.ds(r0, ocut[n] - r0)
        return pltpu.make_async_copy(obuf.at[r, :], o_w.at[r, :], sem_o.at[n])

    def loop_c(i, carry):
        mm_sp_out(i, [], True)
        pl.when(i == NB - 2)(cp_o(0).start)
        return carry

    with jax.named_scope("sec_c"):
        jax.lax.fori_loop(0, NB, loop_c, 0)
    for n in range(OSPL):
        cp_o(n + 1).start()
    for n in range(OSPL + 1):
        cp_o(n).wait()


@jax.jit
def pallas_interleave_layers__ssm_conv_h3__mixer_gmlp__prompt_kernel(
    A_q: jax.Array,
    A_k: jax.Array,
    A_v: jax.Array,
    A_shift_k: jax.Array,
    A_ssm_k: jax.Array,
    A_ssm_D: jax.Array,
    B_x: jax.Array,
    B_w_in: jax.Array,
    B_w_sp: jax.Array,
    B_b_sp: jax.Array,
    B_w_out: jax.Array,
):
    del B_x
    hbm = pl.BlockSpec(memory_space=pl.ANY)
    nslot = (NP - 1) * NTILE
    out = pl.pallas_call(
        _kernel,
        out_shape=jax.ShapeDtypeStruct((S, D), BF16),
        in_specs=[hbm] * 11,
        out_specs=hbm,
        scratch_shapes=[
            pltpu.VMEM((NTILE, S // 2 + 8, LANES), U32),
            pltpu.VMEM((NTILE, S // 2, LANES), U32),
            pltpu.VMEM((NTILE, LANES // 2, S), U32),
            pltpu.VMEM((CST_ROWS, LANES), U32),
            pltpu.VMEM(((S + TM) // 2, D), U32),
            pltpu.VMEM((D // 2, F), U32),
            pltpu.VMEM((S // 2, S), U32),
            pltpu.VMEM((FH // 2, D), U32),
            pltpu.VMEM((NTILE, 8, LANES), F32),
            pltpu.VMEM((S, LANES), F32),
            pltpu.VMEM((2, RF, LANES // 2, LANES), U32),
            pltpu.VMEM((2, RF, LANES // 2, LANES), U32),
            pltpu.VMEM((2, RI, LANES // 2, LANES), U32),
            pltpu.VMEM((nslot, 2, RF, 2 * LANES + 8, LANES), F32),
            pltpu.VMEM((NTILE, S + 8, LANES), F32),
            pltpu.VMEM((S + TM, D), F32),
            pltpu.VMEM((S // 2, FH), U32),
            pltpu.VMEM((S // 2, FH), U32),
            pltpu.VMEM((FH // LANES, TM + 8, LANES), F32),
            pltpu.VMEM((TM // 2, FH), U32),
            pltpu.VMEM((TM // 2, D), U32),
            pltpu.VMEM((TM // 2 + 8, D), U32),
            pltpu.VMEM((S // 2, D), U32),
            pltpu.VMEM((8, LANES), U32),
            pltpu.VMEM((KS, D), BF16),
            pltpu.VMEM((NTILE, LANES), BF16),
            pltpu.VMEM((S // LANES, LANES), BF16),
            pltpu.VMEM((S // LANES, LANES), F32),
            pltpu.SMEM((1,), jnp.int32),
            pltpu.SemaphoreType.DMA((NP, NTILE)),
            pltpu.SemaphoreType.DMA((NP, NTILE)),
            pltpu.SemaphoreType.DMA((NP, NTILE)),
            pltpu.SemaphoreType.DMA((5,)),
            pltpu.SemaphoreType.DMA((NB,)),
            pltpu.SemaphoreType.DMA((2 * FH // TN,)),
            pltpu.SemaphoreType.DMA((2,)),
            pltpu.SemaphoreType.DMA((OSPL + 1,)),
        ],
        compiler_params=pltpu.CompilerParams(
            vmem_limit_bytes=120 * 1024 * 1024),
    )(
        A_q.reshape(S, D), A_k.reshape(S, D), A_v.reshape(S, D),
        A_shift_k.T, A_ssm_k, A_ssm_D.reshape(NTILE, LANES),
        B_w_in, B_w_sp, B_b_sp.reshape(S // LANES, LANES), B_w_out,
        jnp.asarray(_constants()),
    )
    return out.reshape(1, S, D)
```
